```python
import os as _os
_os.environ.setdefault("JAX_PLATFORMS", "cpu")
import jax
import jax.numpy as jnp

def _softmax(x, axis=-1):
    return jax.nn.softmax(x, axis=axis)
def _gelu(x):
    return jax.nn.gelu(x, approximate=True)
def _silu(x):
    return jax.nn.silu(x)
def _sigmoid(x):
    return jax.nn.sigmoid(x)
def _layernorm(x, axis=-1, eps=1e-5):
    m = jnp.mean(x, axis=axis, keepdims=True)
    v = jnp.var(x, axis=axis, keepdims=True)
    return (x - m) / jnp.sqrt(v + eps)
def _scatter_add(tgt, idx, src, axis=0):
    return tgt.at[idx].add(src)
def _segment_sum(src, seg, n):
    return jax.ops.segment_sum(src, seg, n)
class _Rng:
    def __init__(self, key):
        self._k = key
    def _next(self):
        self._k, sub = jax.random.split(self._k)
        return sub
    def normal(self, shape):
        return jax.random.normal(self._next(), shape, dtype=jnp.bfloat16)
    def randint(self, lo, hi, shape):
        return jax.random.randint(self._next(), shape, lo, hi, dtype=jnp.int32)
    def uniform(self, shape, lo=0.0, hi=1.0):
        return jax.random.uniform(self._next(), shape, jnp.bfloat16, lo, hi)
    def permutation(self, n):
        return jax.random.permutation(self._next(), n)


kernel_name = 'gated_mix__linear_kernel_hedgehog__glu_gated_bilinear__prompt'

def setup_inputs():
    _rng = _Rng(jax.random.key(int.from_bytes(__import__("os").urandom(4), "little")))
    _w = (lambda a: (lambda t: t.astype(jnp.bfloat16) if jnp.issubdtype(t.dtype, jnp.floating) else t)(jnp.asarray(a)))
    def _A_setup():
        B, S, D, H = 1, 2048, 512, 32
        Dh = D // H
        return {
            "x": _w((lambda *s: _rng.normal(s) * 0.05)(B, S, D)),
            "wqkv": _w((lambda *s: _rng.normal(s) * 0.8)(D, 3 * D)),
            "w_phi": _w((lambda *s: _rng.normal(s) * 0.8)(H, Dh, Dh) * (Dh ** -0.5)),
            "wo": _w((lambda *s: _rng.normal(s) * 0.05)(D, D)),
        }
    _A_in = _A_setup()

    def _B_setup():
        B, S, D, F = 1, 2048, 512, 1792
        return {
            "x": _w((lambda *s: _rng.normal(s) * 0.05)(B, S, D)),
            "w_gate": _w((lambda *s: _rng.normal(s) * 1.6)(D, F) * (D ** -0.5)),
            "w_up": _w((lambda *s: _rng.normal(s) * 1.6)(D, F) * (D ** -0.5)),
            "w_down": _w((lambda *s: _rng.normal(s) * 1.6)(F, D) * (F ** -0.5)),
        }
    _B_in = _B_setup()

    return {
        "A_x": _A_in["x"],
        "A_wqkv": _A_in["wqkv"],
        "A_w_phi": _A_in["w_phi"],
        "A_wo": _A_in["wo"],
        "B_x": _B_in["x"],
        "B_w_gate": _B_in["w_gate"],
        "B_w_up": _B_in["w_up"],
        "B_w_down": _B_in["w_down"],
        "gate_w": _w((lambda *s: _rng.normal(s) * 0.05)(512) * 16.0),
    }

def reference(A_x, A_wqkv, A_w_phi, A_wo, B_x, B_w_gate, B_w_up, B_w_down, gate_w):
    def _A_ref(x, wqkv, w_phi, wo):
        B, S, D = x.shape
        H = 32; Dh = D // H
        qkv = (lambda x, *d: x.transpose(*d))((x @ wqkv).reshape(B, S, 3, H, Dh), 2, 0, 3, 1, 4)
        q, k, v = qkv[0], qkv[1], qkv[2]
        pq = jnp.einsum("bhsd,hdf->bhsf", q, w_phi)
        pk = jnp.einsum("bhsd,hdf->bhsf", k, w_phi)
        phi_q = jnp.concatenate([_softmax(pq, axis=-1), _softmax(-pq, axis=-1)], axis=-1)
        phi_k = jnp.concatenate([_softmax(pk, axis=-1), _softmax(-pk, axis=-1)], axis=-1)
        kv = jnp.einsum("bhsf,bhsd->bhfd", phi_k, v)
        z  = jnp.einsum("bhsf->bhf", phi_k)
        num = jnp.einsum("bhqf,bhfd->bhqd", phi_q, kv)
        den = jnp.einsum("bhqf,bhf->bhq", phi_q, z)[..., None] + 1e-6
        o = num / den
        return (lambda x, *d: x.transpose(*d))(o, 0, 2, 1, 3).reshape(B, S, D) @ wo

    def _B_ref(x, w_gate, w_up, w_down):
        g = jnp.einsum("bsd,df->bsf", x, w_gate)
        u = jnp.einsum("bsd,df->bsf", x, w_up)
        h = g * u
        return jnp.einsum("bsf,fd->bsd", h, w_down)

    x = A_x
    g = _sigmoid((x * gate_w).sum(-1, keepdims=True))
    a = _A_ref(x, A_wqkv, A_w_phi, A_wo)
    b = _B_ref(x, B_w_gate, B_w_up, B_w_down)
    return g * a + (1 - g) * b
```

```python
import functools
import jax
import jax.numpy as jnp
from jax import lax
import jax.experimental.pallas as pl
import jax.experimental.pallas.tpu as pltpu

S, D, H, DH, F = 2048, 512, 32, 16, 1792
NB = D // 128
NT_DIMS = (((1,), (1,)), ((), ()))
f32 = jnp.float32
bf16 = jnp.bfloat16


def _nt(a, b):
    return lax.dot_general(a, b, NT_DIMS, preferred_element_type=f32)


def _nn(a, b):
    return jnp.dot(a, b, preferred_element_type=f32)


def _softmax_pair(p):
    mx = jnp.max(p, axis=0, keepdims=True)
    mn = jnp.min(p, axis=0, keepdims=True)
    ep = jnp.exp(p - mx)
    en = jnp.exp(mn - p)
    rp = 1.0 / jnp.sum(ep, axis=0, keepdims=True)
    rn = 1.0 / jnp.sum(en, axis=0, keepdims=True)
    return ep, en, rp, rn


def make(T1=512, T2=512, FC=256, U1=0, U2=0):
    n1 = S // T1
    n2 = S // T2
    nF = F // FC
    NX = 4
    XC = S // NX

    def kernel(x_hbm, wqkv_hbm, wphi_hbm, wo_hbm, wg_hbm, wu_hbm, wd_hbm, gw_hbm, o_hbm,
               x_v, wqkv_v, wphi_v, wo_v, wg_v, wu_v, wd_v, gw_v, out_v,
               wkT_s, wqT_s, kv_acc, z_acc, kvT_bf, z_col, sems, xsems, osems):

        def cp(src, dst, k):
            return pltpu.make_async_copy(src, dst, sems.at[k])

        def part(p):
            return cp(wqkv_hbm.at[:, p * D:(p + 1) * D], wqkv_v.at[:, p * D:(p + 1) * D], p)

        def xcp(t):
            return pltpu.make_async_copy(x_hbm.at[pl.ds(t * XC, XC)], x_v.at[pl.ds(t * XC, XC)], xsems.at[t])

        def ocp(t):
            return pltpu.make_async_copy(out_v.at[pl.ds(t * T2, T2)], o_hbm.at[pl.ds(t * T2, T2)], osems.at[t])

        c_phi = cp(wphi_hbm, wphi_v, 3)
        c_gw = cp(gw_hbm, gw_v, 4)
        c_wg = cp(wg_hbm, wg_v, 5)
        c_wu = cp(wu_hbm, wu_v, 6)
        c_wd = cp(wd_hbm, wd_v, 7)
        c_wo = cp(wo_hbm, wo_v, 8)

        c_phi.start()
        part(1).start()
        xcp(0).start()
        part(2).start()
        for t in range(1, NX):
            xcp(t).start()
        c_gw.start()
        part(0).start()
        c_wg.start()
        c_wu.start()
        c_wd.start()
        c_wo.start()

        kv_acc[...] = jnp.zeros_like(kv_acc)
        z_acc[...] = jnp.zeros_like(z_acc)

        c_phi.wait()
        m2 = wphi_v[...].reshape(DH * DH, H)
        r = lax.broadcasted_iota(jnp.int32, (H, D), 0)
        c = lax.broadcasted_iota(jnp.int32, (H, D), 1)
        eh = jnp.where(r == (c >> 4), 1.0, 0.0).astype(bf16)
        m3 = _nn(m2, eh)
        r = lax.broadcasted_iota(jnp.int32, (DH * DH, D), 0)
        c = lax.broadcasted_iota(jnp.int32, (DH * DH, D), 1)
        m3 = jnp.where((r >> 4) == (c & 15), m3, 0.0).astype(bf16)
        r = lax.broadcasted_iota(jnp.int32, (128, DH * DH), 0)
        c = lax.broadcasted_iota(jnp.int32, (128, DH * DH), 1)
        er = jnp.where((r >> 3) == (c & 15), 1.0, 0.0).astype(bf16)
        a_all = _nn(er, m3)
        r2 = lax.broadcasted_iota(jnp.int32, (128, D), 0)
        c2 = lax.broadcasted_iota(jnp.int32, (128, D), 1)
        a_all = jnp.where((r2 & 7) == ((c2 >> 4) & 7), a_all, 0.0).astype(bf16)

        part(1).wait()
        for j in range(NB):
            a_j = a_all[:, 128 * j:128 * (j + 1)]
            wk_j = wqkv_v[:, D + 128 * j:D + 128 * (j + 1)]
            wkT_s[128 * j:128 * (j + 1), :] = _nt(a_j, wk_j).astype(bf16)
        part(2).wait()

        def phase1(t, carry):
            TS = T1
            if T1 >= XC:
                for u in range(T1 // XC):
                    xcp(t * (T1 // XC) + u).wait()
            else:
                @pl.when(t % (XC // T1) == 0)
                def _():
                    xcp(t // (XC // T1)).wait()
            off = pl.multiple_of(t * TS, TS)
            x = x_v[pl.ds(off, TS), :]
            pkT = _nt(wkT_s[...], x)
            v = _nn(x, wqkv_v[:, 2 * D:3 * D]).astype(bf16)
            for j in range(NB):
                p = pkT[128 * j:128 * (j + 1), :].reshape(DH, 8, TS)
                ep, en, rp, rn = _softmax_pair(p)
                php = (ep * rp).reshape(128, TS)
                phn = (en * rn).reshape(128, TS)
                ph = jnp.concatenate([php, phn], axis=0)
                zp = ph[:, 0:128]
                for u in range(1, TS // 128):
                    zp = zp + ph[:, 128 * u:128 * (u + 1)]
                z_acc[j] += zp
                kv_acc[j] += _nn(ph.astype(bf16), v[:, 128 * j:128 * (j + 1)])
            return carry

        if U1:
            for t in range(n1):
                phase1(t, 0)
        else:
            lax.fori_loop(0, n1, phase1, 0)

        part(0).wait()
        for j in range(NB):
            a_j = a_all[:, 128 * j:128 * (j + 1)]
            wq_j = wqkv_v[:, 128 * j:128 * (j + 1)]
            wqT_s[128 * j:128 * (j + 1), :] = _nt(a_j, wq_j).astype(bf16)

        r = lax.broadcasted_iota(jnp.int32, (256, 128), 0)
        c = lax.broadcasted_iota(jnp.int32, (256, 128), 1)
        mask = (r & 7) == (c >> 4)
        for j in range(NB):
            kvm = jnp.where(mask, kv_acc[j], 0.0)
            kvT_bf[j] = kvm.T.astype(bf16)
            z_col[j] = jnp.broadcast_to(jnp.sum(z_acc[j], axis=1, keepdims=True), (256, 128))
        c_gw.wait()
        c_wg.wait()
        c_wu.wait()
        c_wd.wait()
        c_wo.wait()

        def phase2(t, carry):
            TS = T2
            off = pl.multiple_of(t * TS, TS)
            x = x_v[pl.ds(off, TS), :]
            pqT = _nt(wqT_s[...], x)

            def attn(j):
                p = pqT[128 * j:128 * (j + 1), :].reshape(DH, 8, TS)
                ep, en, rp, rn = _softmax_pair(p)
                zc = z_col[j]
                zc = jnp.concatenate([zc] * (TS // 128), axis=1)
                zp = zc[0:128].reshape(DH, 8, TS)
                zn = zc[128:256].reshape(DH, 8, TS)
                tp = jnp.sum(ep * zp, axis=0, keepdims=True)
                tn = jnp.sum(en * zn, axis=0, keepdims=True)
                den = tp * rp + tn * rn + 1e-6
                inv = 1.0 / den
                php = (ep * (rp * inv)).reshape(128, TS)
                phn = (en * (rn * inv)).reshape(128, TS)
                ph = jnp.concatenate([php.astype(bf16), phn.astype(bf16)], axis=0)
                oT = _nn(kvT_bf[j], ph)
                return oT.astype(bf16).T

            def ffn(c):
                gg = _nn(x, wg_v[:, FC * c:FC * (c + 1)])
                uu = _nn(x, wu_v[:, FC * c:FC * (c + 1)])
                h = (gg * uu).astype(bf16)
                return _nn(h, wd_v[FC * c:FC * (c + 1), :])

            os_ = []
            b = None
            for c in range(nF):
                bb = ffn(c)
                b = bb if b is None else b + bb
                if c < NB:
                    os_.append(attn(c))
            for j in range(nF, NB):
                os_.append(attn(j))
            o = jnp.concatenate(os_, axis=1)
            a = _nn(o, wo_v[...])
            gl = jnp.sum(x.astype(f32) * gw_v[...].astype(f32).reshape(1, D), axis=1, keepdims=True)
            g = 1.0 / (1.0 + jnp.exp(-gl))
            out_v[pl.ds(off, TS), :] = (g * a + (1.0 - g) * b).astype(out_v.dtype)
            ocp(t).start()
            return carry

        if U2:
            for t in range(n2):
                phase2(t, 0)
        else:
            lax.fori_loop(0, n2, phase2, 0)
        for t in range(n2):
            ocp(t).wait()

    @jax.jit
    def fn(A_x, A_wqkv, A_w_phi, A_wo, B_x, B_w_gate, B_w_up, B_w_down, gate_w):
        x2 = A_x.reshape(S, D)
        wphi_t = jnp.transpose(A_w_phi, (1, 2, 0))
        any_spec = pl.BlockSpec(memory_space=pl.ANY)
        out = pl.pallas_call(
            kernel,
            in_specs=[any_spec] * 8,
            out_specs=any_spec,
            out_shape=jax.ShapeDtypeStruct((S, D), bf16),
            scratch_shapes=[
                pltpu.VMEM((S, D), bf16),
                pltpu.VMEM((D, 3 * D), bf16),
                pltpu.VMEM((DH, DH, H), bf16),
                pltpu.VMEM((D, D), bf16),
                pltpu.VMEM((D, F), bf16),
                pltpu.VMEM((D, F), bf16),
                pltpu.VMEM((F, D), bf16),
                pltpu.VMEM((D,), bf16),
                pltpu.VMEM((S, D), bf16),
                pltpu.VMEM((D, D), bf16),
                pltpu.VMEM((D, D), bf16),
                pltpu.VMEM((NB, 256, 128), f32),
                pltpu.VMEM((NB, 256, 128), f32),
                pltpu.VMEM((NB, 128, 256), bf16),
                pltpu.VMEM((NB, 256, 128), f32),
                pltpu.SemaphoreType.DMA((9,)),
                pltpu.SemaphoreType.DMA((NX,)),
                pltpu.SemaphoreType.DMA((n2,)),
            ],
            compiler_params=pltpu.CompilerParams(
                vmem_limit_bytes=100 * 1024 * 1024,
            ),
        )(x2, A_wqkv, wphi_t, A_wo, B_w_gate, B_w_up, B_w_down, gate_w)
        return out.reshape(1, S, D)

    return fn


pallas_gated_mix__linear_kernel_hedgehog__glu_gated_bilinear__prompt_kernel = make(T1=512, T2=512)
```

```python
import contextlib
import functools
import jax
import jax.numpy as jnp
from jax import lax
import jax.experimental.pallas as pl
import jax.experimental.pallas.tpu as pltpu

S, D, H, DH, F = 2048, 512, 32, 16, 1792
NB = D // 128
NG = 8
NT_DIMS = (((1,), (1,)), ((), ()))
f32 = jnp.float32
bf16 = jnp.bfloat16
LOG2E = 1.4426950408889634


def _nt(a, b):
    return lax.dot_general(a, b, NT_DIMS, preferred_element_type=f32)


def _nn(a, b):
    return jnp.dot(a, b, preferred_element_type=f32)


def _lhs7(a11, a12, a21, a22):
    f = [a.astype(f32) for a in (a11, a12, a21, a22)]
    return [(f[0] + f[3]).astype(bf16), (f[2] + f[3]).astype(bf16), a11.astype(bf16), a22.astype(bf16),
            (f[0] + f[1]).astype(bf16), (f[2] - f[0]).astype(bf16), (f[1] - f[3]).astype(bf16)]


def _rhs7(b11, b12, b21, b22):
    f = [b.astype(f32) for b in (b11, b12, b21, b22)]
    return [(f[0] + f[3]).astype(bf16), b11, (f[1] - f[3]).astype(bf16), (f[2] - f[0]).astype(bf16),
            b22, (f[0] + f[1]).astype(bf16), (f[2] + f[3]).astype(bf16)]


def _rhs7_lazy(g11, g12, g21, g22):
    def add(a, b):
        return lambda: (a().astype(f32) + b().astype(f32)).astype(bf16)

    def sub(a, b):
        return lambda: (a().astype(f32) - b().astype(f32)).astype(bf16)
    return [add(g11, g22), g11, sub(g12, g22), sub(g21, g11), g22, add(g11, g12), add(g21, g22)]


def _lhs7_lazy(g11, g12, g21, g22):
    def add(a, b):
        return lambda: (a().astype(f32) + b().astype(f32)).astype(bf16)

    def sub(a, b):
        return lambda: (a().astype(f32) - b().astype(f32)).astype(bf16)
    return [add(g11, g22), add(g21, g22), g11, g22, add(g11, g12), sub(g21, g11), sub(g12, g22)]


def _comb(m):
    c11 = (m[0] + m[3]) + (m[6] - m[4])
    c12 = m[2] + m[4]
    c21 = m[1] + m[3]
    c22 = (m[0] - m[1]) + (m[2] + m[5])
    return [c11, c12, c21, c22]


def make(T2=1024, RC=128, E2=1, SC=0, RCP=1, ORD=1, SV=1, WV=0, OT32=1, LZ=0, DM=2, DLAG=0, PB=32, CO=0):
    T1 = 512
    n1 = S // T1
    n2 = S // T2
    NX = 4
    XC = S // NX
    NO = S // RC
    _exp = jnp.exp2 if E2 else jnp.exp
    PORD = (1, 4, 0, 2, 3, 5, 6) if ORD else tuple(range(7))

    def _prod7(la, lb):
        m = [None] * 7
        for i in PORD:
            m[i] = _nn(la[i], lb[i]() if callable(lb[i]) else lb[i])
        return m

    def scope(name):
        return jax.named_scope(name) if SC else contextlib.nullcontext()

    def _rcp(x):
        if RCP == 0:
            return 1.0 / x
        r = pl.reciprocal(x, approx=True)
        if RCP == 2:
            r = r * (2.0 - x * r)
        return r

    def _red(x, red, op):
        y = red(x, axis=0)
        y = op(y, pltpu.roll(y, 4, 0))
        return y[None]

    def _softmax_pair(p):
        mx = _red(p, jnp.max, jnp.maximum)
        mn = _red(p, jnp.min, jnp.minimum)
        ep = _exp(p - mx)
        en = _exp(mn - p)
        rp = _rcp(_red(ep, jnp.sum, jnp.add))
        rn = _rcp(_red(en, jnp.sum, jnp.add))
        return ep, en, rp, rn

    def kernel(x_hbm, wqkv_hbm, wphi_hbm, wo_hbm, wg_hbm, wu_hbm, wd_hbm, gw_hbm, o_hbm,
               x_v, wqkv_v, wphi_v, wo_v, wg_v, wu_v, wd_v, gw_v, out_v,
               wkT_s, wqT_s, kv_bf, z_col, xs_s, sems, xsems, osems):

        def cp(src, dst, k):
            return pltpu.make_async_copy(src, dst, sems.at[k])

        def part(p):
            return cp(wqkv_hbm.at[:, p * D:(p + 1) * D], wqkv_v.at[:, p * D:(p + 1) * D], p)

        def xcp(t):
            return pltpu.make_async_copy(x_hbm.at[pl.ds(t * XC, XC)], x_v.at[pl.ds(t * XC, XC)], xsems.at[t])

        def ocp(t):
            return pltpu.make_async_copy(out_v.at[pl.ds(t * RC, RC)], o_hbm.at[pl.ds(t * RC, RC)], osems.at[t])

        c_phi = cp(wphi_hbm, wphi_v, 3)
        c_gw = cp(gw_hbm, gw_v, 4)
        c_wg = cp(wg_hbm, wg_v, 5)
        c_wu = cp(wu_hbm, wu_v, 6)
        c_wd = cp(wd_hbm, wd_v, 7)
        c_wo = cp(wo_hbm, wo_v, 8)

        c_phi.start()
        part(1).start()
        xcp(0).start()

        with scope('w_phi'):
            c_phi.wait()
        m2 = wphi_v[...].reshape(DH * DH, H)
        r = lax.broadcasted_iota(jnp.int32, (H, D), 0)
        c = lax.broadcasted_iota(jnp.int32, (H, D), 1)
        eh = jnp.where(r == (c >> 4), 1.0, 0.0).astype(bf16)
        m3 = _nn(m2, eh)
        r = lax.broadcasted_iota(jnp.int32, (DH * DH, D), 0)
        c = lax.broadcasted_iota(jnp.int32, (DH * DH, D), 1)
        m3 = jnp.where((r >> 4) == (c & 15), m3, 0.0).astype(bf16)
        r = lax.broadcasted_iota(jnp.int32, (128, DH * DH), 0)
        c = lax.broadcasted_iota(jnp.int32, (128, DH * DH), 1)
        er = jnp.where(((r >> 2) & 15) == (c & 15), 1.0, 0.0).astype(bf16)
        a_all = _nn(er, m3)
        r2 = lax.broadcasted_iota(jnp.int32, (128, D), 0)
        c2 = lax.broadcasted_iota(jnp.int32, (128, D), 1)
        a_all = jnp.where((((r2 >> 6) << 2) | (r2 & 3)) == ((c2 >> 4) & 7), a_all, 0.0).astype(bf16)

        def fold(p, dst):
            for j in range(NB):
                a_j = a_all[:, 128 * j:128 * (j + 1)]
                w_j = wqkv_v[:, p * D + 128 * j:p * D + 128 * (j + 1)]
                w = _nt(a_j, w_j)
                if E2:
                    w = w * LOG2E
                dst[128 * j:128 * (j + 1), :] = w.astype(bf16)

        def xtile(t):
            return x_v[pl.ds(t * T1, T1), :]

        def kphi(t):
            TS = T1
            pkT = _nt(wkT_s[...], xtile(t))
            phs, zs = [], []
            for g in range(NG):
                p = pkT[64 * g:64 * (g + 1), :].reshape(8, 8, TS)
                ep, en, rp, rn = _softmax_pair(p)
                ph = jnp.concatenate([ep * rp, en * rn], axis=0).reshape(128, TS)
                zp = ph[:, 0:128]
                for u in range(1, TS // 128):
                    zp = zp + ph[:, 128 * u:128 * (u + 1)]
                zs.append(zp)
                phs.append(ph.astype(bf16))
            return phs, zs

        SUMS = (0, 1, 4, 5, 6)

        def xprep(tt):
            for rb in range(512 // PB):
                r0 = 1024 * tt + PB * rb
                top = x_v[r0:r0 + PB, :]
                bot = x_v[r0 + 512:r0 + 512 + PB, :]
                LA = _lhs7(top[:, :256], top[:, 256:], bot[:, :256], bot[:, 256:])
                for k, i in enumerate(SUMS):
                    xs_s[tt, k, PB * rb:PB * (rb + 1), :] = LA[i]

        def load_la(tt, off):
            LA = [None] * 7
            for k, i in enumerate(SUMS):
                LA[i] = xs_s[tt, k]
            LA[2] = x_v[pl.ds(off, 512), 0:256]
            LA[3] = x_v[pl.ds(off + 512, 512), 256:512]
            return LA

        def vproj2(tt):
            if SV:
                LA = load_la(tt, 1024 * tt)
                o2 = 2 * D
                LB = _rhs7(wqkv_v[:256, o2:o2 + 256], wqkv_v[:256, o2 + 256:o2 + 512],
                           wqkv_v[256:, o2:o2 + 256], wqkv_v[256:, o2 + 256:o2 + 512])
                C = [cc.astype(bf16) for cc in _comb(_prod7(LA, LB))]
                vs = [jnp.concatenate([C[0], C[1]], axis=1), jnp.concatenate([C[2], C[3]], axis=1)]
            else:
                vs = [_nn(xtile(2 * tt + u), wqkv_v[:, 2 * D:3 * D]).astype(bf16) for u in range(2)]
            return [[v[:, 128 * j:128 * (j + 1)].T for j in range(NB)] for v in vs]

        def kvm(vT, phs):
            kvs = []
            for g in range(NG):
                vg = vT[g // 2][64 * (g % 2):64 * (g % 2 + 1), :]
                kvs.append(_nt(vg, phs[g]))
            return kvs

        def acc(lst, new):
            return new if lst is None else [a + b for a, b in zip(lst, new)]

        with scope('w_wk'):
            part(1).wait()
        part(2).start()
        c_gw.start()
        with scope('foldk'):
            fold(1, wkT_s)
        with scope('w_x0'):
            xcp(0).wait()
        xcp(1).start()
        with scope('kphi0'):
            phs0, zs = kphi(0)
        with scope('w_wv'):
            part(2).wait()
            xcp(1).wait()
            c_gw.wait()
        for t in range(2, NX):
            xcp(t).start()
        part(0).start()
        c_wg.start()
        c_wu.start()
        with scope('blkB'):
            xprep(0)
            phs1, zs1 = kphi(1)
            zs = acc(zs, zs1)
            vT = vproj2(0)
            kvs = acc(kvm(vT[0], phs0), kvm(vT[1], phs1))
        with scope('w_x23'):
            xcp(2).wait()
            xcp(3).wait()
            part(0).wait()
        c_wd.start()
        c_wo.start()
        with scope('blkC'):
            xprep(1)
            phs0, zs1 = kphi(2)
            zs = acc(zs, zs1)
            if CO == 0:
                phs1, zs1 = kphi(3)
                zs = acc(zs, zs1)
                vT = vproj2(1)
                kvs = acc(kvs, acc(kvm(vT[0], phs0), kvm(vT[1], phs1)))
                fold(0, wqT_s)
                wqT_s[D:D + 16, :] = jnp.broadcast_to(gw_v[...].astype(f32).reshape(1, D), (16, D)).astype(bf16)
            else:
                vT = vproj2(1)
                phs1, zs1 = kphi(3)
                zs = acc(zs, zs1)
                kvs = acc(kvs, kvm(vT[0], phs0))
                fold(0, wqT_s)
                kvs = acc(kvs, kvm(vT[1], phs1))
            r = lax.broadcasted_iota(jnp.int32, (64, 128), 0)
            c = lax.broadcasted_iota(jnp.int32, (64, 128), 1)
            mask = (r >> 4) == (c & 3)
            for g in range(NG):
                kv_bf[g] = jnp.where(mask, kvs[g], 0.0).astype(bf16)
                z_col[g] = jnp.broadcast_to(jnp.sum(zs[g], axis=1, keepdims=True), (128, 128))

        with scope('w_big'):
            c_wg.wait()
            c_wu.wait()
            c_wd.wait()
            c_wo.wait()

        def phase2(t, carry):
            with scope('p2body'):
                return phase2_(t, carry)

        def phase2_(t, carry):
            TS = T2
            R = TS // 2
            off = pl.multiple_of(t * TS, TS)
            x = x_v[pl.ds(off, TS), :]
            pqT = _nt(wqT_s[...], x)
            gT = 1.0 / (1.0 + jnp.exp(-pqT[D:D + 8, :]))
            ngT = 1.0 - gT
            ngate_b = jnp.concatenate(
                [jnp.concatenate([ngT[:, 128 * u:128 * (u + 1)]] * 16, axis=0).T for u in range(TS // 128)], axis=0)

            def attn(g):
                p = pqT[64 * g:64 * (g + 1), :].reshape(8, 8, TS)
                ep, en, rp, rn = _softmax_pair(p)
                zc = z_col[g]
                zc = jnp.concatenate([zc] * (TS // 128), axis=1)
                zp = zc[0:64].reshape(8, 8, TS)
                zn = zc[64:128].reshape(8, 8, TS)
                tp = jnp.sum(ep * zp, axis=0, keepdims=True)
                tn = jnp.sum(en * zn, axis=0, keepdims=True)
                den = _red(tp * rp + tn * rn, jnp.sum, jnp.add) + 1e-6
                inv = _rcp(den) * gT[None]
                ph = jnp.concatenate([ep * (rp * inv), en * (rn * inv)], axis=0).reshape(128, TS).astype(bf16)
                return _nn(kv_bf[g], ph)

            def attn2(j):
                oa = attn(j)
                ob = attn(j + 4)
                return _lhs7(oa[:, :R], ob[:, :R], oa[:, R:], ob[:, R:])

            os_ = []
            LA = load_la(t, off)
            LHs = []
            NS = None

            def ldc(c):
                c0, c1, c2 = 256 * c, 256 * c + 128, 256 * c + 256
                return _rhs7(wd_v[c0:c1, :256], wd_v[c0:c1, 256:], wd_v[c1:c2, :256], wd_v[c1:c2, 256:])

            def down(cs, NS):
                LDs = [ldc(c) for c in cs]
                m = [None] * 7
                for i in PORD:
                    acc_ = None if NS is None else NS[i]
                    for k, c in enumerate(cs):
                        p_ = _nn(LHs[c][i], LDs[k][i])
                        acc_ = p_ if acc_ is None else acc_ + p_
                    m[i] = acc_
                return m

            pend = []
            for c in range(7):
                c0, c1, c2 = 256 * c, 256 * c + 128, 256 * c + 256

                def blk(r0, ca, cb):
                    return jnp.concatenate([wg_v[r0:r0 + 256, ca:cb], wu_v[r0:r0 + 256, ca:cb]], axis=1)
                LB = _rhs7(blk(0, c0, c1), blk(0, c1, c2), blk(256, c0, c1), blk(256, c1, c2))
                C = _comb(_prod7(LA, LB))
                if DLAG and pend and len(pend) >= DM:
                    NS = down(pend, NS)
                    pend = []
                sc = [ngate_b[:R], ngate_b[:R], ngate_b[R:], ngate_b[R:]]
                hs = [(cc[:, :128] * cc[:, 128:]) * s_ for cc, s_ in zip(C, sc)]
                LHs.append(_lhs7(*hs))
                pend.append(c)
                if c < NB:
                    os_.append(attn2(c))
                if not DLAG and len(pend) >= DM:
                    NS = down(pend, NS)
                    pend = []
            if pend:
                NS = down(pend, NS)

            LO = [jnp.concatenate([jnp.concatenate([os_[2 * k][i], os_[2 * k + 1][i]], axis=0).T for k in range(2)], axis=1)
                  for i in range(7)]
            if LZ >= 2:
                LW = [f() for f in _rhs7_lazy(lambda: wo_v[:256, :256], lambda: wo_v[:256, 256:],
                                              lambda: wo_v[256:, :256], lambda: wo_v[256:, 256:])]
            else:
                LW = _rhs7(wo_v[:256, :256], wo_v[:256, 256:], wo_v[256:, :256], wo_v[256:, 256:])
            for p in range(R // RC):
                sl = slice(p * RC, (p + 1) * RC)
                P = _prod7([lo[sl] for lo in LO], LW)
                C = _comb([n[sl] + q for n, q in zip(NS, P)])
                top = jnp.concatenate([C[0], C[1]], axis=1).astype(out_v.dtype)
                bot = jnp.concatenate([C[2], C[3]], axis=1).astype(out_v.dtype)
                out_v[pl.ds(pl.multiple_of(off + p * RC, RC), RC), :] = top
                out_v[pl.ds(pl.multiple_of(off + R + p * RC, RC), RC), :] = bot
                ocp(t * (TS // RC) + p).start()
                ocp(t * (TS // RC) + R // RC + p).start()
            return carry

        lax.fori_loop(0, n2, phase2, 0)
        with scope('w_out'):
            for t in range(NO):
                ocp(t).wait()

    @jax.jit
    def fn(A_x, A_wqkv, A_w_phi, A_wo, B_x, B_w_gate, B_w_up, B_w_down, gate_w):
        x2 = A_x.reshape(S, D)
        wphi_t = jnp.transpose(A_w_phi, (1, 2, 0))
        any_spec = pl.BlockSpec(memory_space=pl.ANY)
        out = pl.pallas_call(
            kernel,
            in_specs=[any_spec] * 8,
            out_specs=any_spec,
            out_shape=jax.ShapeDtypeStruct((S, D), bf16),
            scratch_shapes=[
                pltpu.VMEM((S, D), bf16),
                pltpu.VMEM((D, 3 * D), bf16),
                pltpu.VMEM((DH, DH, H), bf16),
                pltpu.VMEM((D, D), bf16),
                pltpu.VMEM((D, F), bf16),
                pltpu.VMEM((D, F), bf16),
                pltpu.VMEM((F, D), bf16),
                pltpu.VMEM((D,), bf16),
                pltpu.VMEM((S, D), bf16),
                pltpu.VMEM((D, D), bf16),
                pltpu.VMEM((D + 16, D), bf16),
                pltpu.VMEM((NG, 64, 128), bf16),
                pltpu.VMEM((NG, 128, 128), f32),
                pltpu.VMEM((2, 5, 512, 256), bf16),
                pltpu.SemaphoreType.DMA((9,)),
                pltpu.SemaphoreType.DMA((NX,)),
                pltpu.SemaphoreType.DMA((NO,)),
            ],
            compiler_params=pltpu.CompilerParams(
                vmem_limit_bytes=100 * 1024 * 1024,
            ),
        )(x2, A_wqkv, wphi_t, A_wo, B_w_gate, B_w_up, B_w_down, gate_w)
        return out.reshape(1, S, D)

    return fn


pallas_gated_mix__linear_kernel_hedgehog__glu_gated_bilinear__prompt_kernel = make(PB=128)
```

```python
import jax
import jax.numpy as jnp
from jax import lax
import jax.experimental.pallas as pl
import jax.experimental.pallas.tpu as pltpu

S, D, H, DH, F = 2048, 512, 32, 16, 1792
NB = D // 128
NG = 8
T1 = 512
T2 = 1024
R = T2 // 2
NF = F // 256
PCS = (192, 160, 96, 64)
POFF = (0, 192, 352, 448)
PORD = (4, 1, 2, 3, 0, 5, 6)
XSUMS = (0, 1, 4, 5, 6)
NT_DIMS = (((1,), (1,)), ((), ()))
LOG2E = 1.4426950408889634
f32 = jnp.float32
bf16 = jnp.bfloat16


def _nt(a, b):
    return lax.dot_general(a, b, NT_DIMS, preferred_element_type=f32)


def _nn(a, b):
    return jnp.dot(a, b, preferred_element_type=f32)


def _lhs7(a11, a12, a21, a22):
    f = [a.astype(f32) for a in (a11, a12, a21, a22)]
    return [(f[0] + f[3]).astype(bf16), (f[2] + f[3]).astype(bf16), a11.astype(bf16), a22.astype(bf16),
            (f[0] + f[1]).astype(bf16), (f[2] - f[0]).astype(bf16), (f[1] - f[3]).astype(bf16)]


def _rhs7(b11, b12, b21, b22):
    f = [b.astype(f32) for b in (b11, b12, b21, b22)]
    return [(f[0] + f[3]).astype(bf16), b11, (f[1] - f[3]).astype(bf16), (f[2] - f[0]).astype(bf16),
            b22, (f[0] + f[1]).astype(bf16), (f[2] + f[3]).astype(bf16)]


def _prod7(la, lb):
    m = [None] * 7
    for i in PORD:
        m[i] = _nn(la[i], lb[i])
    return m


def _comb(m):
    c11 = (m[0] + m[3]) + (m[6] - m[4])
    c12 = m[2] + m[4]
    c21 = m[1] + m[3]
    c22 = (m[0] - m[1]) + (m[2] + m[5])
    return [c11, c12, c21, c22]


def _red(x, red, op):
    y = red(x, axis=0)
    y = op(y, pltpu.roll(y, 4, 0))
    return y[None]


def _rcp(x):
    return pl.reciprocal(x, approx=True)


def _softmax_pair(p):
    mx = _red(p, jnp.max, jnp.maximum)
    mn = _red(p, jnp.min, jnp.minimum)
    ep = jnp.exp2(p - mx)
    en = jnp.exp2(mn - p)
    rp = _rcp(_red(ep, jnp.sum, jnp.add))
    rn = _rcp(_red(en, jnp.sum, jnp.add))
    return ep, en, rp, rn


def _acc(lst, new):
    return [a + b for a, b in zip(lst, new)]


def _kernel(x_hbm, wqkv_hbm, wphi_hbm, wo_hbm, wg_hbm, wu_hbm, wd_hbm, gw_hbm, o_hbm,
            x_v, wqkv_v, wphi_v, wo_v, wg_v, wu_v, wd_v, gw_v, out_v,
            wkT_s, wqT_s, kv_bf, z_col, xs_s, sems):

    def cp(src, dst, k):
        return pltpu.make_async_copy(src, dst, sems.at[k])

    def part(p):
        k = {0: 1, 1: 1, 2: 0}[p]
        return cp(wqkv_hbm.at[:, p * D:(p + 1) * D], wqkv_v.at[:, p * D:(p + 1) * D], k)

    def xcp(t):
        k = {0: 2, 1: 0, 2: 1, 3: 1}[t]
        return cp(x_hbm.at[pl.ds(t * T1, T1)], x_v.at[pl.ds(t * T1, T1)], k)

    def ocp(t, p, half):
        r0 = pl.multiple_of(t * T2 + half * R + POFF[p], 16)
        return cp(out_v.at[pl.ds(r0, PCS[p])], o_hbm.at[pl.ds(r0, PCS[p])], 0)

    c_phi = cp(wphi_hbm, wphi_v, 0)
    c_gw = cp(gw_hbm, gw_v, 0)
    c_wg = cp(wg_hbm, wg_v, 2)
    c_wu = cp(wu_hbm, wu_v, 2)
    c_wd = cp(wd_hbm, wd_v, 2)
    c_wo = cp(wo_hbm, wo_v, 2)

    c_phi.start()
    part(1).start()
    xcp(0).start()

    c_phi.wait()
    m2 = wphi_v[...].reshape(DH * DH, H)
    r = lax.broadcasted_iota(jnp.int32, (H, D), 0)
    c = lax.broadcasted_iota(jnp.int32, (H, D), 1)
    eh = jnp.where(r == (c >> 4), 1.0, 0.0).astype(bf16)
    m3 = _nn(m2, eh)
    r = lax.broadcasted_iota(jnp.int32, (DH * DH, D), 0)
    c = lax.broadcasted_iota(jnp.int32, (DH * DH, D), 1)
    m3 = jnp.where((r >> 4) == (c & 15), m3, 0.0).astype(bf16)
    r = lax.broadcasted_iota(jnp.int32, (128, DH * DH), 0)
    c = lax.broadcasted_iota(jnp.int32, (128, DH * DH), 1)
    er = jnp.where(((r >> 2) & 15) == (c & 15), 1.0, 0.0).astype(bf16)
    a_all = _nn(er, m3)
    r = lax.broadcasted_iota(jnp.int32, (128, D), 0)
    c = lax.broadcasted_iota(jnp.int32, (128, D), 1)
    a_all = jnp.where((((r >> 6) << 2) | (r & 3)) == ((c >> 4) & 7), a_all, 0.0).astype(bf16)

    def fold(p, dst, r0):
        for j in range(NB):
            w = _nt(a_all[:, 128 * j:128 * (j + 1)], wqkv_v[:, p * D + 128 * j:p * D + 128 * (j + 1)])
            dst[r0 + 128 * j:r0 + 128 * (j + 1), :] = (w * LOG2E).astype(bf16)

    def xtile(t):
        return x_v[t * T1:(t + 1) * T1, :]

    def ksoft(pkT):
        ts = pkT.shape[1]
        phs, zs = [], []
        for g in range(NG):
            p = pkT[64 * g:64 * (g + 1), :].reshape(8, 8, ts)
            ep, en, rp, rn = _softmax_pair(p)
            ph = jnp.concatenate([ep * rp, en * rn], axis=0).reshape(128, ts)
            zp = ph[:, 0:128]
            for u in range(1, ts // 128):
                zp = zp + ph[:, 128 * u:128 * (u + 1)]
            zs.append(zp)
            phs.append(ph.astype(bf16))
        return phs, zs

    def kphi(t):
        return ksoft(_nt(wkT_s[...], xtile(t)))

    def xprep(tt):
        for rb in range(R // 128):
            r0 = T2 * tt + 128 * rb
            top = x_v[r0:r0 + 128, :]
            bot = x_v[r0 + R:r0 + R + 128, :]
            la = _lhs7(top[:, :256], top[:, 256:], bot[:, :256], bot[:, 256:])
            for k, i in enumerate(XSUMS):
                xs_s[tt, k, 128 * rb:128 * (rb + 1), :] = la[i]

    def load_la(tt, off):
        la = [None] * 7
        for k, i in enumerate(XSUMS):
            la[i] = xs_s[tt, k]
        la[2] = x_v[pl.ds(off, R), 0:256]
        la[3] = x_v[pl.ds(off + R, R), 256:512]
        return la

    def vproj2(tt):
        o2 = 2 * D
        lb = _rhs7(wqkv_v[:256, o2:o2 + 256], wqkv_v[:256, o2 + 256:o2 + 512],
                   wqkv_v[256:, o2:o2 + 256], wqkv_v[256:, o2 + 256:o2 + 512])
        cs = [cc.astype(bf16) for cc in _comb(_prod7(load_la(tt, T2 * tt), lb))]
        vs = [jnp.concatenate([cs[0], cs[1]], axis=1), jnp.concatenate([cs[2], cs[3]], axis=1)]
        return [[v[:, 128 * j:128 * (j + 1)].T for j in range(NB)] for v in vs]

    def kvm(vT, phs):
        return [_nt(vT[g // 2][64 * (g % 2):64 * (g % 2 + 1), :], phs[g]) for g in range(NG)]

    part(1).wait()
    part(2).start()
    c_gw.start()
    fold(1, wkT_s, 0)
    xcp(0).wait()
    xcp(1).start()

    pk0 = _nt(wkT_s[...], xtile(0))
    phs0, zs = ksoft(pk0[:, :T1 - 128])

    part(2).wait()
    xcp(1).wait()
    c_gw.wait()
    xcp(2).start()
    xcp(3).start()
    part(0).start()
    c_wg.start()
    c_wu.start()

    phs0b, zs0b = ksoft(pk0[:, T1 - 128:])
    phs0 = [jnp.concatenate([a, b], axis=1) for a, b in zip(phs0, phs0b)]
    zs = _acc(zs, zs0b)
    xprep(0)
    phs1, zs1 = kphi(1)
    zs = _acc(zs, zs1)
    vT = vproj2(0)
    kvs = _acc(kvm(vT[0], phs0), kvm(vT[1], phs1))

    xcp(2).wait()
    xcp(3).wait()
    part(0).wait()
    c_wd.start()
    c_wo.start()

    xprep(1)
    phs0, zs1 = kphi(2)
    zs = _acc(zs, zs1)
    phs1, zs1 = kphi(3)
    zs = _acc(zs, zs1)
    vT = vproj2(1)
    kvs = _acc(kvs, _acc(kvm(vT[0], phs0), kvm(vT[1], phs1)))
    fold(0, wqT_s, 16)
    wqT_s[0:16, :] = jnp.broadcast_to(gw_v[...].astype(f32).reshape(1, D), (16, D)).astype(bf16)
    r = lax.broadcasted_iota(jnp.int32, (64, 128), 0)
    c = lax.broadcasted_iota(jnp.int32, (64, 128), 1)
    same_head = (r >> 4) == (c & 3)
    for g in range(NG):
        kv_bf[g] = jnp.where(same_head, kvs[g], 0.0).astype(bf16)
        z_col[g] = jnp.broadcast_to(jnp.sum(zs[g], axis=1, keepdims=True), (128, 128))

    c_wg.wait()
    c_wu.wait()
    c_wd.wait()
    c_wo.wait()

    def phase2(t, carry):
        off = pl.multiple_of(t * T2, T2)
        x = x_v[pl.ds(off, T2), :]
        pqT = _nt(wqT_s[...], x)
        gT = 1.0 / (1.0 + jnp.exp(-pqT[0:8, :]))
        ngT = 1.0 - gT
        ngate = jnp.concatenate(
            [jnp.concatenate([ngT[:, 128 * u:128 * (u + 1)]] * 16, axis=0).T for u in range(T2 // 128)],
            axis=0)

        def attn(g):
            p = pqT[16 + 64 * g:16 + 64 * (g + 1), :].reshape(8, 8, T2)
            ep, en, rp, rn = _softmax_pair(p)
            zc = jnp.concatenate([z_col[g]] * (T2 // 128), axis=1)
            tp = jnp.sum(ep * zc[0:64].reshape(8, 8, T2), axis=0, keepdims=True)
            tn = jnp.sum(en * zc[64:128].reshape(8, 8, T2), axis=0, keepdims=True)
            den = _red(tp * rp + tn * rn, jnp.sum, jnp.add) + 1e-6
            inv = _rcp(den) * gT[None]
            ph = jnp.concatenate([ep * (rp * inv), en * (rn * inv)], axis=0).reshape(128, T2).astype(bf16)
            return _nn(kv_bf[g], ph)

        def attn2(j):
            oa = attn(j)
            ob = attn(j + 4)
            return _lhs7(oa[:, :R], ob[:, :R], oa[:, R:], ob[:, R:])

        la = load_la(t, off)
        lhs_h, os_ = [], []

        def down(cs, ns):
            lds = []
            for c_ in cs:
                c0, c1, c2 = 256 * c_, 256 * c_ + 128, 256 * c_ + 256
                lds.append(_rhs7(wd_v[c0:c1, :256], wd_v[c0:c1, 256:], wd_v[c1:c2, :256], wd_v[c1:c2, 256:]))
            m = [None] * 7
            for i in PORD:
                a = None if ns is None else ns[i]
                for k, c_ in enumerate(cs):
                    q = _nn(lhs_h[c_][i], lds[k][i])
                    a = q if a is None else a + q
                m[i] = a
            return m

        ns = None
        pend = []
        for c_ in range(NF):
            c0, c1, c2 = 256 * c_, 256 * c_ + 128, 256 * c_ + 256

            def blk(r0, ca, cb):
                return jnp.concatenate([wg_v[r0:r0 + 256, ca:cb], wu_v[r0:r0 + 256, ca:cb]], axis=1)
            lb = _rhs7(blk(0, c0, c1), blk(0, c1, c2), blk(256, c0, c1), blk(256, c1, c2))
            gu = _comb(_prod7(la, lb))
            sc = [ngate[:R], ngate[:R], ngate[R:], ngate[R:]]
            lhs_h.append(_lhs7(*[(b[:, :128] * b[:, 128:]) * s for b, s in zip(gu, sc)]))
            pend.append(c_)
            if c_ < NB:
                os_.append(attn2(c_))
            if len(pend) == 2:
                ns = down(pend, ns)
                pend = []
        ns = down(pend, ns)

        lo = [jnp.concatenate([jnp.concatenate([os_[2 * k][i], os_[2 * k + 1][i]], axis=0).T for k in range(2)],
                              axis=1) for i in range(7)]
        lw = _rhs7(wo_v[:256, :256], wo_v[:256, 256:], wo_v[256:, :256], wo_v[256:, 256:])
        for p in range(len(PCS)):
            sl = slice(POFF[p], POFF[p] + PCS[p])
            pr = _prod7([a[sl] for a in lo], lw)
            cb = _comb([n[sl] + q for n, q in zip(ns, pr)])
            top = jnp.concatenate([cb[0], cb[1]], axis=1).astype(out_v.dtype)
            bot = jnp.concatenate([cb[2], cb[3]], axis=1).astype(out_v.dtype)
            out_v[pl.ds(pl.multiple_of(off + POFF[p], 16), PCS[p]), :] = top
            out_v[pl.ds(pl.multiple_of(off + R + POFF[p], 16), PCS[p]), :] = bot
            ocp(t, p, 0).start()
            ocp(t, p, 1).start()
        return carry

    lax.fori_loop(0, S // T2, phase2, 0)
    cp(out_v, o_hbm, 0).wait()


@jax.jit
def pallas_gated_mix__linear_kernel_hedgehog__glu_gated_bilinear__prompt_kernel(
    A_x: jax.Array,
    A_wqkv: jax.Array,
    A_w_phi: jax.Array,
    A_wo: jax.Array,
    B_x: jax.Array,
    B_w_gate: jax.Array,
    B_w_up: jax.Array,
    B_w_down: jax.Array,
    gate_w: jax.Array,
):
    del B_x
    x2 = A_x.reshape(S, D)
    wphi_t = jnp.transpose(A_w_phi, (1, 2, 0))
    any_spec = pl.BlockSpec(memory_space=pl.ANY)
    out = pl.pallas_call(
        _kernel,
        in_specs=[any_spec] * 8,
        out_specs=any_spec,
        out_shape=jax.ShapeDtypeStruct((S, D), bf16),
        scratch_shapes=[
            pltpu.VMEM((S, D), bf16),
            pltpu.VMEM((D, 3 * D), bf16),
            pltpu.VMEM((DH, DH, H), bf16),
            pltpu.VMEM((D, D), bf16),
            pltpu.VMEM((D, F), bf16),
            pltpu.VMEM((D, F), bf16),
            pltpu.VMEM((F, D), bf16),
            pltpu.VMEM((D,), bf16),
            pltpu.VMEM((S, D), bf16),
            pltpu.VMEM((D, D), bf16),
            pltpu.VMEM((D + 16, D), bf16),
            pltpu.VMEM((NG, 64, 128), bf16),
            pltpu.VMEM((NG, 128, 128), f32),
            pltpu.VMEM((2, 5, R, 256), bf16),
            pltpu.SemaphoreType.DMA((3,)),
        ],
        compiler_params=pltpu.CompilerParams(vmem_limit_bytes=100 * 1024 * 1024),
    )(x2, A_wqkv, wphi_t, A_wo, B_w_gate, B_w_up, B_w_down, gate_w)
    return out.reshape(1, S, D)
```

```python
import jax
import jax.numpy as jnp
from jax import lax
import jax.experimental.pallas as pl
import jax.experimental.pallas.tpu as pltpu

S, D, H, DH, F = 2048, 512, 32, 16, 1792
NB = D // 128
NG = 8
T1 = 512
T2 = 1024
R = T2 // 2
NF = F // 256
PCS = (192, 160, 96, 64)
POFF = (0, 192, 352, 448)
PORD = (4, 1, 2, 3, 0, 5, 6)
XSUMS = (0, 1, 4, 5, 6)
NR = 480
NT_DIMS = (((1,), (1,)), ((), ()))
LOG2E = 1.4426950408889634
f32 = jnp.float32
bf16 = jnp.bfloat16


def _nt(a, b):
    return lax.dot_general(a, b, NT_DIMS, preferred_element_type=f32)


def _nn(a, b):
    return jnp.dot(a, b, preferred_element_type=f32)


def _lhs7(a11, a12, a21, a22):
    f = [a.astype(f32) for a in (a11, a12, a21, a22)]
    return [(f[0] + f[3]).astype(bf16), (f[2] + f[3]).astype(bf16), a11.astype(bf16), a22.astype(bf16),
            (f[0] + f[1]).astype(bf16), (f[2] - f[0]).astype(bf16), (f[1] - f[3]).astype(bf16)]


def _rhs7(b11, b12, b21, b22):
    f = [b.astype(f32) for b in (b11, b12, b21, b22)]
    return [(f[0] + f[3]).astype(bf16), b11, (f[1] - f[3]).astype(bf16), (f[2] - f[0]).astype(bf16),
            b22, (f[0] + f[1]).astype(bf16), (f[2] + f[3]).astype(bf16)]


def _prod7(la, lb):
    m = [None] * 7
    for i in PORD:
        m[i] = _nn(la[i], lb[i])
    return m


def _comb(m):
    c11 = (m[0] + m[3]) + (m[6] - m[4])
    c12 = m[2] + m[4]
    c21 = m[1] + m[3]
    c22 = (m[0] - m[1]) + (m[2] + m[5])
    return [c11, c12, c21, c22]


def _red(x, red, op):
    y = red(x, axis=0)
    y = op(y, pltpu.roll(y, 4, 0))
    return y[None]


def _rcp(x):
    return pl.reciprocal(x, approx=True)


def _softmax_pair(p):
    mx = _red(p, jnp.max, jnp.maximum)
    mn = _red(p, jnp.min, jnp.minimum)
    ep = jnp.exp2(p - mx)
    en = jnp.exp2(mn - p)
    rp = _rcp(_red(ep, jnp.sum, jnp.add))
    rn = _rcp(_red(en, jnp.sum, jnp.add))
    return ep, en, rp, rn


def _acc(lst, new):
    return [a + b for a, b in zip(lst, new)]


def _kernel(x_hbm, wqkv_hbm, wphi_hbm, wo_hbm, wg_hbm, wu_hbm, wd_hbm, gw_hbm, o_hbm,
            x_v, wq_v, wk_v, wv_v, wphi_v, wo_v, wg_v, wu_v, wd_v, gw_v, out_v,
            wkT_s, wqT_s, kv_bf, z_col, xs_s, sems):

    def cp(src, dst, k):
        return pltpu.make_async_copy(src, dst, sems.at[k])

    def part(p):
        k = {0: 1, 1: 1, 2: 0}[p]
        return cp(wqkv_hbm.at[:, p * D:(p + 1) * D], (wq_v, wk_v, wv_v)[p], k)

    def xcp(t):
        k = {0: 2, 1: 0, 2: 1, 3: 1}[t]
        return cp(x_hbm.at[pl.ds(t * T1, T1)], x_v.at[pl.ds(t * T1, T1)], k)

    def ocp(t, p, half):
        r0 = pl.multiple_of(t * T2 + half * R + POFF[p], 16)
        return cp(out_v.at[pl.ds(r0, PCS[p])], o_hbm.at[pl.ds(r0, PCS[p])], 0)

    c_phi = cp(wphi_hbm, wphi_v, 0)
    c_gw = cp(gw_hbm, gw_v, 0)
    c_wg = cp(wg_hbm, wg_v, 2)
    c_wu = cp(wu_hbm, wu_v, 2)
    c_wd = cp(wd_hbm, wd_v, 2)
    c_wo = cp(wo_hbm, wo_v, 2)

    c_phi.start()
    part(1).start()
    xcp(0).start()

    c_phi.wait()
    m2 = wphi_v[...].reshape(DH * DH, H)
    r = lax.broadcasted_iota(jnp.int32, (H, D), 0)
    c = lax.broadcasted_iota(jnp.int32, (H, D), 1)
    eh = jnp.where(r == (c >> 4), 1.0, 0.0).astype(bf16)
    m3 = _nn(m2, eh)
    r = lax.broadcasted_iota(jnp.int32, (DH * DH, D), 0)
    c = lax.broadcasted_iota(jnp.int32, (DH * DH, D), 1)
    m3 = jnp.where((r >> 4) == (c & 15), m3, 0.0).astype(bf16)
    r = lax.broadcasted_iota(jnp.int32, (128, DH * DH), 0)
    c = lax.broadcasted_iota(jnp.int32, (128, DH * DH), 1)
    er = jnp.where(((r >> 2) & 15) == (c & 15), 1.0, 0.0).astype(bf16)
    a_all = _nn(er, m3)
    r = lax.broadcasted_iota(jnp.int32, (128, D), 0)
    c = lax.broadcasted_iota(jnp.int32, (128, D), 1)
    a_all = jnp.where((((r >> 6) << 2) | (r & 3)) == ((c >> 4) & 7), a_all, 0.0).astype(bf16)

    def fold(w_ref, dst, r0):
        lo_half = lax.broadcasted_iota(jnp.int32, (8, D), 0) < 4
        rows = []
        for j in range(NB):
            w = _nt(a_all[:, 128 * j:128 * (j + 1)], w_ref[:, 128 * j:128 * (j + 1)]) * LOG2E
            last, full = [], []
            for gl in range(2):
                wg_ = w[64 * gl:64 * (gl + 1)].reshape(8, 8, D)
                s7 = wg_[7]
                s7r = pltpu.roll(s7, 4, 0)
                ref = jnp.where(lo_half, s7r, s7) if gl == 0 else jnp.where(lo_half, s7, s7r)
                full.append((wg_[0:7] - ref[None]).reshape(56, D))
                last.append(s7 - ref)
            rows.append(jnp.where(lo_half, last[0], last[1]))
            rows.extend(full)
        dst[r0:r0 + NR, :] = jnp.concatenate(rows, axis=0).astype(bf16)

    def logits(pT, g):
        ts = pT.shape[1]
        base = 120 * (g // 2)
        full = pT[base + 8 + 56 * (g % 2):base + 8 + 56 * (g % 2 + 1), :].reshape(7, 8, ts)
        lo_half = lax.broadcasted_iota(jnp.int32, (8, ts), 0) < 4
        keep = lo_half if g % 2 == 0 else jnp.logical_not(lo_half)
        s7 = jnp.where(keep, pT[base:base + 8, :], 0.0)
        return jnp.concatenate([full, s7[None]], axis=0)

    def xtile(t):
        return x_v[t * T1:(t + 1) * T1, :]

    def ksoft(pkT):
        ts = pkT.shape[1]
        phs, zs = [], []
        for g in range(NG):
            p = logits(pkT, g)
            ep, en, rp, rn = _softmax_pair(p)
            ph = jnp.concatenate([ep * rp, en * rn], axis=0).reshape(128, ts)
            zp = ph[:, 0:128]
            for u in range(1, ts // 128):
                zp = zp + ph[:, 128 * u:128 * (u + 1)]
            zs.append(zp)
            phs.append(ph.astype(bf16))
        return phs, zs

    def kphi(t):
        return ksoft(_nt(wkT_s[...], xtile(t)))

    def xprep(tt):
        for rb in range(R // 128):
            r0 = T2 * tt + 128 * rb
            top = x_v[r0:r0 + 128, :]
            bot = x_v[r0 + R:r0 + R + 128, :]
            la = _lhs7(top[:, :256], top[:, 256:], bot[:, :256], bot[:, 256:])
            for k, i in enumerate(XSUMS):
                xs_s[tt, k, 128 * rb:128 * (rb + 1), :] = la[i]

    def load_la(tt, off):
        la = [None] * 7
        for k, i in enumerate(XSUMS):
            la[i] = xs_s[tt, k]
        la[2] = x_v[pl.ds(off, R), 0:256]
        la[3] = x_v[pl.ds(off + R, R), 256:512]
        return la

    def vproj2(tt):
        lb = _rhs7(wv_v[:256, :256], wv_v[:256, 256:], wv_v[256:, :256], wv_v[256:, 256:])
        cs = [cc.astype(bf16) for cc in _comb(_prod7(load_la(tt, T2 * tt), lb))]
        vs = [jnp.concatenate([cs[0], cs[1]], axis=1), jnp.concatenate([cs[2], cs[3]], axis=1)]
        return [[v[:, 128 * j:128 * (j + 1)].T for j in range(NB)] for v in vs]

    def kvm(vT, phs):
        return [_nt(vT[g // 2][64 * (g % 2):64 * (g % 2 + 1), :], phs[g]) for g in range(NG)]

    part(1).wait()
    part(2).start()
    c_gw.start()
    fold(wk_v, wkT_s, 0)
    xcp(0).wait()
    xcp(1).start()

    pk0 = _nt(wkT_s[...], xtile(0))
    phs0, zs = ksoft(pk0[:, :T1 - 128])

    part(2).wait()
    xcp(1).wait()
    c_gw.wait()
    xcp(2).start()
    xcp(3).start()
    part(0).start()
    c_wg.start()
    c_wu.start()

    phs0b, zs0b = ksoft(pk0[:, T1 - 128:])
    phs0 = [jnp.concatenate([a, b], axis=1) for a, b in zip(phs0, phs0b)]
    zs = _acc(zs, zs0b)
    xprep(0)
    phs1, zs1 = kphi(1)
    zs = _acc(zs, zs1)
    vT = vproj2(0)
    kvs = _acc(kvm(vT[0], phs0), kvm(vT[1], phs1))

    xcp(2).wait()
    xcp(3).wait()
    part(0).wait()
    c_wd.start()
    c_wo.start()

    xprep(1)
    phs0, zs1 = kphi(2)
    zs = _acc(zs, zs1)
    phs1, zs1 = kphi(3)
    zs = _acc(zs, zs1)
    vT = vproj2(1)
    kvs = _acc(kvs, _acc(kvm(vT[0], phs0), kvm(vT[1], phs1)))
    fold(wq_v, wqT_s, 16)
    wqT_s[0:16, :] = jnp.broadcast_to(gw_v[...].astype(f32).reshape(1, D), (16, D)).astype(bf16)
    r = lax.broadcasted_iota(jnp.int32, (64, 128), 0)
    c = lax.broadcasted_iota(jnp.int32, (64, 128), 1)
    same_head = (r >> 4) == (c & 3)
    for g in range(NG):
        kv_bf[g] = jnp.where(same_head, kvs[g], 0.0).astype(bf16)
        z_col[g] = jnp.broadcast_to(jnp.sum(zs[g], axis=1, keepdims=True), (128, 128))

    c_wg.wait()
    c_wu.wait()
    c_wd.wait()
    c_wo.wait()

    def phase2(t, carry):
        off = pl.multiple_of(t * T2, T2)
        x = x_v[pl.ds(off, T2), :]
        pqT = _nt(wqT_s[...], x)
        gT = 1.0 / (1.0 + jnp.exp(-pqT[0:8, :]))
        ngT = 1.0 - gT
        ngate = jnp.concatenate(
            [jnp.concatenate([ngT[:, 128 * u:128 * (u + 1)]] * 16, axis=0).T for u in range(T2 // 128)],
            axis=0)

        def attn(g):
            p = logits(pqT[16:], g)
            ep, en, rp, rn = _softmax_pair(p)
            zc = jnp.concatenate([z_col[g]] * (T2 // 128), axis=1)
            tp = jnp.sum(ep * zc[0:64].reshape(8, 8, T2), axis=0, keepdims=True)
            tn = jnp.sum(en * zc[64:128].reshape(8, 8, T2), axis=0, keepdims=True)
            den = _red(tp * rp + tn * rn, jnp.sum, jnp.add) + 1e-6
            inv = _rcp(den) * gT[None]
            ph = jnp.concatenate([ep * (rp * inv), en * (rn * inv)], axis=0).reshape(128, T2).astype(bf16)
            return _nn(kv_bf[g], ph)

        def attn2(j):
            oa = attn(j)
            ob = attn(j + 4)
            return _lhs7(oa[:, :R], ob[:, :R], oa[:, R:], ob[:, R:])

        la = load_la(t, off)
        lhs_h, os_ = [], []

        def down(cs, ns):
            lds = []
            for c_ in cs:
                c0, c1, c2 = 256 * c_, 256 * c_ + 128, 256 * c_ + 256
                lds.append(_rhs7(wd_v[c0:c1, :256], wd_v[c0:c1, 256:], wd_v[c1:c2, :256], wd_v[c1:c2, 256:]))
            m = [None] * 7
            for i in PORD:
                a = None if ns is None else ns[i]
                for k, c_ in enumerate(cs):
                    q = _nn(lhs_h[c_][i], lds[k][i])
                    a = q if a is None else a + q
                m[i] = a
            return m

        ns = None
        pend = []
        for c_ in range(NF):
            c0, c1, c2 = 256 * c_, 256 * c_ + 128, 256 * c_ + 256

            def blk(r0, ca, cb):
                return jnp.concatenate([wg_v[r0:r0 + 256, ca:cb], wu_v[r0:r0 + 256, ca:cb]], axis=1)
            lb = _rhs7(blk(0, c0, c1), blk(0, c1, c2), blk(256, c0, c1), blk(256, c1, c2))
            gu = _comb(_prod7(la, lb))
            sc = [ngate[:R], ngate[:R], ngate[R:], ngate[R:]]
            lhs_h.append(_lhs7(*[(b[:, :128] * b[:, 128:]) * s for b, s in zip(gu, sc)]))
            pend.append(c_)
            if c_ < NB:
                os_.append(attn2(c_))
            if len(pend) == 2:
                ns = down(pend, ns)
                pend = []
        ns = down(pend, ns)

        lo = [jnp.concatenate([jnp.concatenate([os_[2 * k][i], os_[2 * k + 1][i]], axis=0).T for k in range(2)],
                              axis=1) for i in range(7)]
        lw = _rhs7(wo_v[:256, :256], wo_v[:256, 256:], wo_v[256:, :256], wo_v[256:, 256:])
        for p in range(len(PCS)):
            sl = slice(POFF[p], POFF[p] + PCS[p])
            pr = _prod7([a[sl] for a in lo], lw)
            cb = _comb([n[sl] + q for n, q in zip(ns, pr)])
            top = jnp.concatenate([cb[0], cb[1]], axis=1).astype(out_v.dtype)
            bot = jnp.concatenate([cb[2], cb[3]], axis=1).astype(out_v.dtype)
            out_v[pl.ds(pl.multiple_of(off + POFF[p], 16), PCS[p]), :] = top
            out_v[pl.ds(pl.multiple_of(off + R + POFF[p], 16), PCS[p]), :] = bot
            ocp(t, p, 0).start()
            ocp(t, p, 1).start()
        return carry

    lax.fori_loop(0, S // T2, phase2, 0)
    cp(out_v, o_hbm, 0).wait()


@jax.jit
def pallas_gated_mix__linear_kernel_hedgehog__glu_gated_bilinear__prompt_kernel(
    A_x: jax.Array,
    A_wqkv: jax.Array,
    A_w_phi: jax.Array,
    A_wo: jax.Array,
    B_x: jax.Array,
    B_w_gate: jax.Array,
    B_w_up: jax.Array,
    B_w_down: jax.Array,
    gate_w: jax.Array,
):
    del B_x
    x2 = A_x.reshape(S, D)
    wphi_t = jnp.transpose(A_w_phi, (1, 2, 0))
    any_spec = pl.BlockSpec(memory_space=pl.ANY)
    out = pl.pallas_call(
        _kernel,
        in_specs=[any_spec] * 8,
        out_specs=any_spec,
        out_shape=jax.ShapeDtypeStruct((S, D), bf16),
        scratch_shapes=[
            pltpu.VMEM((S, D), bf16),
            pltpu.VMEM((D, D), bf16),
            pltpu.VMEM((D, D), bf16),
            pltpu.VMEM((D, D), bf16),
            pltpu.VMEM((DH, DH, H), bf16),
            pltpu.VMEM((D, D), bf16),
            pltpu.VMEM((D, F), bf16),
            pltpu.VMEM((D, F), bf16),
            pltpu.VMEM((F, D), bf16),
            pltpu.VMEM((D,), bf16),
            pltpu.VMEM((S, D), bf16),
            pltpu.VMEM((NR, D), bf16),
            pltpu.VMEM((NR + 16, D), bf16),
            pltpu.VMEM((NG, 64, 128), bf16),
            pltpu.VMEM((NG, 128, 128), f32),
            pltpu.VMEM((2, 5, R, 256), bf16),
            pltpu.SemaphoreType.DMA((3,)),
        ],
        compiler_params=pltpu.CompilerParams(vmem_limit_bytes=100 * 1024 * 1024),
    )(x2, A_wqkv, wphi_t, A_wo, B_w_gate, B_w_up, B_w_down, gate_w)
    return out.reshape(1, S, D)
```

```python
import jax
import jax.numpy as jnp
from jax import lax
import jax.experimental.pallas as pl
import jax.experimental.pallas.tpu as pltpu

S, D, H, DH, F = 2048, 512, 32, 16, 1792
NB = D // 128
NG = 8
T1 = 512
T2 = 1024
R = T2 // 2
NF = F // 256
PCS = (192, 160, 96, 64)
POFF = (0, 192, 352, 448)
PORD = (4, 1, 2, 3, 0, 5, 6)
XSUMS = (0, 1, 4, 5, 6)
NT_DIMS = (((1,), (1,)), ((), ()))
LOG2E = 1.4426950408889634
f32 = jnp.float32
bf16 = jnp.bfloat16


def _nt(a, b):
    return lax.dot_general(a, b, NT_DIMS, preferred_element_type=f32)


def _nn(a, b):
    return jnp.dot(a, b, preferred_element_type=f32)


def _lhs7(a11, a12, a21, a22):
    f = [a.astype(f32) for a in (a11, a12, a21, a22)]
    return [(f[0] + f[3]).astype(bf16), (f[2] + f[3]).astype(bf16), a11.astype(bf16), a22.astype(bf16),
            (f[0] + f[1]).astype(bf16), (f[2] - f[0]).astype(bf16), (f[1] - f[3]).astype(bf16)]


def _rhs7(b11, b12, b21, b22):
    f = [b.astype(f32) for b in (b11, b12, b21, b22)]
    return [(f[0] + f[3]).astype(bf16), b11, (f[1] - f[3]).astype(bf16), (f[2] - f[0]).astype(bf16),
            b22, (f[0] + f[1]).astype(bf16), (f[2] + f[3]).astype(bf16)]


def _prod7(la, lb):
    m = [None] * 7
    for i in PORD:
        m[i] = _nn(la[i], lb[i])
    return m


def _comb(m):
    c11 = (m[0] + m[3]) + (m[6] - m[4])
    c12 = m[2] + m[4]
    c21 = m[1] + m[3]
    c22 = (m[0] - m[1]) + (m[2] + m[5])
    return [c11, c12, c21, c22]


def _red(x, red, op):
    y = red(x, axis=0)
    y = op(y, pltpu.roll(y, 4, 0))
    return y[None]


def _rcp(x):
    return pl.reciprocal(x, approx=True)


def _softmax_pair(p):
    mx = _red(p, jnp.max, jnp.maximum)
    mn = _red(p, jnp.min, jnp.minimum)
    ep = jnp.exp2(p - mx)
    en = jnp.exp2(mn - p)
    rp = _rcp(_red(ep, jnp.sum, jnp.add))
    rn = _rcp(_red(en, jnp.sum, jnp.add))
    return ep, en, rp, rn


def _acc(lst, new):
    return [a + b for a, b in zip(lst, new)]


def _kernel(x_hbm, wqkv_hbm, wphi_hbm, wo_hbm, wg_hbm, wu_hbm, wd_hbm, gw_hbm, o_hbm,
            x_v, wq_v, wk_v, wv_v, wphi_v, wo_v, wg_v, wu_v, wd_v, gw_v, out_v,
            wkT_s, wqT_s, kv_bf, z_col, xs_s, sems):

    def cp(src, dst, k):
        return pltpu.make_async_copy(src, dst, sems.at[k])

    def part(p):
        k = {0: 1, 1: 1, 2: 0}[p]
        return cp(wqkv_hbm.at[:, p * D:(p + 1) * D], (wq_v, wk_v, wv_v)[p], k)

    def xcp(t):
        k = {0: 2, 1: 0, 2: 1, 3: 1}[t]
        return cp(x_hbm.at[pl.ds(t * T1, T1)], x_v.at[pl.ds(t * T1, T1)], k)

    def ocp(t, p, half):
        r0 = pl.multiple_of(t * T2 + half * R + POFF[p], 16)
        return cp(out_v.at[pl.ds(r0, PCS[p])], o_hbm.at[pl.ds(r0, PCS[p])], 0)

    c_phi = cp(wphi_hbm, wphi_v, 0)
    c_gw = cp(gw_hbm, gw_v, 0)
    c_wg = cp(wg_hbm, wg_v, 2)
    c_wu = cp(wu_hbm, wu_v, 2)
    c_wd = cp(wd_hbm, wd_v, 2)
    c_wo = cp(wo_hbm, wo_v, 2)

    c_phi.start()
    part(1).start()
    xcp(0).start()

    c_phi.wait()
    m2 = wphi_v[...].reshape(DH * DH, H)
    r = lax.broadcasted_iota(jnp.int32, (H, D), 0)
    c = lax.broadcasted_iota(jnp.int32, (H, D), 1)
    eh = jnp.where(r == (c >> 4), 1.0, 0.0).astype(bf16)
    m3 = _nn(m2, eh)
    r = lax.broadcasted_iota(jnp.int32, (DH * DH, D), 0)
    c = lax.broadcasted_iota(jnp.int32, (DH * DH, D), 1)
    m3 = jnp.where((r >> 4) == (c & 15), m3, 0.0).astype(bf16)
    r = lax.broadcasted_iota(jnp.int32, (128, DH * DH), 0)
    c = lax.broadcasted_iota(jnp.int32, (128, DH * DH), 1)
    er = jnp.where(((r >> 2) & 15) == (c & 15), 1.0, 0.0).astype(bf16)
    a_all = _nn(er, m3)
    r = lax.broadcasted_iota(jnp.int32, (128, D), 0)
    c = lax.broadcasted_iota(jnp.int32, (128, D), 1)
    a_all = jnp.where((((r >> 6) << 2) | (r & 3)) == ((c >> 4) & 7), a_all, 0.0).astype(bf16)

    def fold(w_ref, dst, r0):
        for j in range(NB):
            w = _nt(a_all[:, 128 * j:128 * (j + 1)], w_ref[:, 128 * j:128 * (j + 1)])
            dst[r0 + 128 * j:r0 + 128 * (j + 1), :] = (w * LOG2E).astype(bf16)

    def xtile(t):
        return x_v[t * T1:(t + 1) * T1, :]

    def ksoft(pkT):
        ts = pkT.shape[1]
        phs, zs = [], []
        for g in range(NG):
            p = pkT[64 * g:64 * (g + 1), :].reshape(8, 8, ts)
            ep, en, rp, rn = _softmax_pair(p)
            ph = jnp.concatenate([ep * rp, en * rn], axis=0).reshape(128, ts)
            zp = ph[:, 0:128]
            for u in range(1, ts // 128):
                zp = zp + ph[:, 128 * u:128 * (u + 1)]
            zs.append(zp)
            phs.append(ph.astype(bf16))
        return phs, zs

    def kphi(t):
        return ksoft(_nt(wkT_s[...], xtile(t)))

    def xprep(tt):
        for rb in range(R // 128):
            r0 = T2 * tt + 128 * rb
            top = x_v[r0:r0 + 128, :]
            bot = x_v[r0 + R:r0 + R + 128, :]
            la = _lhs7(top[:, :256], top[:, 256:], bot[:, :256], bot[:, 256:])
            for k, i in enumerate(XSUMS):
                xs_s[tt, k, 128 * rb:128 * (rb + 1), :] = la[i]

    def load_la(tt, off):
        la = [None] * 7
        for k, i in enumerate(XSUMS):
            la[i] = xs_s[tt, k]
        la[2] = x_v[pl.ds(off, R), 0:256]
        la[3] = x_v[pl.ds(off + R, R), 256:512]
        return la

    def vproj2(tt):
        lb = _rhs7(wv_v[:256, :256], wv_v[:256, 256:], wv_v[256:, :256], wv_v[256:, 256:])
        cs = [cc.astype(bf16) for cc in _comb(_prod7(load_la(tt, T2 * tt), lb))]
        vs = [jnp.concatenate([cs[0], cs[1]], axis=1), jnp.concatenate([cs[2], cs[3]], axis=1)]
        return [[v[:, 128 * j:128 * (j + 1)].T for j in range(NB)] for v in vs]

    def kvm(vT, phs):
        return [_nt(vT[g // 2][64 * (g % 2):64 * (g % 2 + 1), :], phs[g]) for g in range(NG)]

    part(1).wait()
    part(2).start()
    c_gw.start()
    fold(wk_v, wkT_s, 0)
    xcp(0).wait()
    xcp(1).start()

    pk0 = _nt(wkT_s[...], xtile(0))
    phs0, zs = ksoft(pk0[:, :T1 - 128])

    part(2).wait()
    xcp(1).wait()
    c_gw.wait()
    xcp(2).start()
    xcp(3).start()
    part(0).start()
    c_wg.start()
    c_wu.start()

    phs0b, zs0b = ksoft(pk0[:, T1 - 128:])
    phs0 = [jnp.concatenate([a, b], axis=1) for a, b in zip(phs0, phs0b)]
    zs = _acc(zs, zs0b)
    xprep(0)
    phs1, zs1 = kphi(1)
    zs = _acc(zs, zs1)
    vT = vproj2(0)
    kvs = _acc(kvm(vT[0], phs0), kvm(vT[1], phs1))

    xcp(2).wait()
    xcp(3).wait()
    part(0).wait()
    c_wd.start()
    c_wo.start()

    xprep(1)
    phs0, zs1 = kphi(2)
    zs = _acc(zs, zs1)
    phs1, zs1 = kphi(3)
    zs = _acc(zs, zs1)
    vT = vproj2(1)
    kvs = _acc(kvs, _acc(kvm(vT[0], phs0), kvm(vT[1], phs1)))
    fold(wq_v, wqT_s, 16)
    wqT_s[0:16, :] = jnp.broadcast_to(gw_v[...].astype(f32).reshape(1, D), (16, D)).astype(bf16)
    r = lax.broadcasted_iota(jnp.int32, (64, 128), 0)
    c = lax.broadcasted_iota(jnp.int32, (64, 128), 1)
    same_head = (r >> 4) == (c & 3)
    for g in range(NG):
        kv_bf[g] = jnp.where(same_head, kvs[g], 0.0).astype(bf16)
        z_col[g] = jnp.broadcast_to(jnp.sum(zs[g], axis=1, keepdims=True), (128, 128))

    c_wg.wait()
    c_wu.wait()
    c_wd.wait()
    c_wo.wait()

    def phase2(t, carry):
        off = pl.multiple_of(t * T2, T2)
        x = x_v[pl.ds(off, T2), :]
        pqT = _nt(wqT_s[...], x)
        gT = 1.0 / (1.0 + jnp.exp(-pqT[0:8, :]))
        ngT = 1.0 - gT
        ngate = jnp.concatenate(
            [jnp.concatenate([ngT[:, 128 * u:128 * (u + 1)]] * 16, axis=0).T for u in range(T2 // 128)],
            axis=0)

        def attn(g):
            p = pqT[16 + 64 * g:16 + 64 * (g + 1), :].reshape(8, 8, T2)
            ep, en, rp, rn = _softmax_pair(p)
            zc = jnp.concatenate([z_col[g]] * (T2 // 128), axis=1)
            tp = jnp.sum(ep * zc[0:64].reshape(8, 8, T2), axis=0, keepdims=True)
            tn = jnp.sum(en * zc[64:128].reshape(8, 8, T2), axis=0, keepdims=True)
            den = _red(tp * rp + tn * rn, jnp.sum, jnp.add) + 1e-6
            inv = _rcp(den) * gT[None]
            ph = jnp.concatenate([ep * (rp * inv), en * (rn * inv)], axis=0).reshape(128, T2).astype(bf16)
            return _nn(kv_bf[g], ph)

        def attn2(j):
            oa = attn(j)
            ob = attn(j + 4)
            return _lhs7(oa[:, :R], ob[:, :R], oa[:, R:], ob[:, R:])

        la = load_la(t, off)
        lhs_h, os_ = [], []

        def down(cs, ns):
            lds = []
            for c_ in cs:
                c0, c1, c2 = 256 * c_, 256 * c_ + 128, 256 * c_ + 256
                lds.append(_rhs7(wd_v[c0:c1, :256], wd_v[c0:c1, 256:], wd_v[c1:c2, :256], wd_v[c1:c2, 256:]))
            m = [None] * 7
            for i in PORD:
                a = None if ns is None else ns[i]
                for k, c_ in enumerate(cs):
                    q = _nn(lhs_h[c_][i], lds[k][i])
                    a = q if a is None else a + q
                m[i] = a
            return m

        ns = None
        pend = []
        for c_ in range(NF):
            c0, c1, c2 = 256 * c_, 256 * c_ + 128, 256 * c_ + 256

            def blk(r0, ca, cb):
                return jnp.concatenate([wg_v[r0:r0 + 256, ca:cb], wu_v[r0:r0 + 256, ca:cb]], axis=1)
            lb = _rhs7(blk(0, c0, c1), blk(0, c1, c2), blk(256, c0, c1), blk(256, c1, c2))
            gu = _comb(_prod7(la, lb))
            sc = [ngate[:R], ngate[:R], ngate[R:], ngate[R:]]
            lhs_h.append(_lhs7(*[(b[:, :128] * b[:, 128:]) * s for b, s in zip(gu, sc)]))
            pend.append(c_)
            if c_ < NB:
                os_.append(attn2(c_))
            if len(pend) == 2:
                ns = down(pend, ns)
                pend = []
        ns = down(pend, ns)

        lo = [jnp.concatenate([jnp.concatenate([os_[2 * k][i], os_[2 * k + 1][i]], axis=0).T for k in range(2)],
                              axis=1) for i in range(7)]
        lw = _rhs7(wo_v[:256, :256], wo_v[:256, 256:], wo_v[256:, :256], wo_v[256:, 256:])
        for p in range(len(PCS)):
            sl = slice(POFF[p], POFF[p] + PCS[p])
            pr = _prod7([a[sl] for a in lo], lw)
            cb = _comb([n[sl] + q for n, q in zip(ns, pr)])
            top = jnp.concatenate([cb[0], cb[1]], axis=1).astype(out_v.dtype)
            bot = jnp.concatenate([cb[2], cb[3]], axis=1).astype(out_v.dtype)
            out_v[pl.ds(pl.multiple_of(off + POFF[p], 16), PCS[p]), :] = top
            out_v[pl.ds(pl.multiple_of(off + R + POFF[p], 16), PCS[p]), :] = bot
            ocp(t, p, 0).start()
            ocp(t, p, 1).start()
        return carry

    lax.fori_loop(0, S // T2, phase2, 0)
    cp(out_v, o_hbm, 0).wait()


@jax.jit
def pallas_gated_mix__linear_kernel_hedgehog__glu_gated_bilinear__prompt_kernel(
    A_x: jax.Array,
    A_wqkv: jax.Array,
    A_w_phi: jax.Array,
    A_wo: jax.Array,
    B_x: jax.Array,
    B_w_gate: jax.Array,
    B_w_up: jax.Array,
    B_w_down: jax.Array,
    gate_w: jax.Array,
):
    del B_x
    x2 = A_x.reshape(S, D)
    wphi_t = jnp.transpose(A_w_phi, (1, 2, 0))
    any_spec = pl.BlockSpec(memory_space=pl.ANY)
    out = pl.pallas_call(
        _kernel,
        in_specs=[any_spec] * 8,
        out_specs=any_spec,
        out_shape=jax.ShapeDtypeStruct((S, D), bf16),
        scratch_shapes=[
            pltpu.VMEM((S, D), bf16),
            pltpu.VMEM((D, D), bf16),
            pltpu.VMEM((D, D), bf16),
            pltpu.VMEM((D, D), bf16),
            pltpu.VMEM((DH, DH, H), bf16),
            pltpu.VMEM((D, D), bf16),
            pltpu.VMEM((D, F), bf16),
            pltpu.VMEM((D, F), bf16),
            pltpu.VMEM((F, D), bf16),
            pltpu.VMEM((D,), bf16),
            pltpu.VMEM((S, D), bf16),
            pltpu.VMEM((D, D), bf16),
            pltpu.VMEM((D + 16, D), bf16),
            pltpu.VMEM((NG, 64, 128), bf16),
            pltpu.VMEM((NG, 128, 128), f32),
            pltpu.VMEM((2, 5, R, 256), bf16),
            pltpu.SemaphoreType.DMA((3,)),
        ],
        compiler_params=pltpu.CompilerParams(
            vmem_limit_bytes=100 * 1024 * 1024,
            disable_bounds_checks=True,
            disable_semaphore_checks=True,
        ),
    )(x2, A_wqkv, wphi_t, A_wo, B_w_gate, B_w_up, B_w_down, gate_w)
    return out.reshape(1, S, D)
```
